```python
import jax
import jax.numpy as jnp

def _softmax(x, axis=-1):
    return jax.nn.softmax(x, axis=axis)

def _gelu(x):
    return jax.nn.gelu(x, approximate=True)

def _silu(x):
    return jax.nn.silu(x)

def _sigmoid(x):
    return jax.nn.sigmoid(x)

def _layernorm(x, axis=-1, eps=1e-05):
    m = jnp.mean(x, axis=axis, keepdims=True)
    v = jnp.var(x, axis=axis, keepdims=True)
    return (x - m) / jnp.sqrt(v + eps)

def _scatter_add(tgt, idx, src, axis=0):
    return tgt.at[idx].add(src)

def _segment_sum(src, seg, n):
    return jax.ops.segment_sum(src, seg, n)

class _Rng:

    def __init__(self, key):
        self._k = key

    def _next(self):
        self._k, sub = jax.random.split(self._k)
        return sub

    def normal(self, shape):
        return jax.random.normal(self._next(), shape, dtype=jnp.bfloat16)

    def randint(self, lo, hi, shape):
        return jax.random.randint(self._next(), shape, lo, hi, dtype=jnp.int32)

    def uniform(self, shape, lo=0.0, hi=1.0):
        return jax.random.uniform(self._next(), shape, jnp.bfloat16, lo, hi)

    def permutation(self, n):
        return jax.random.permutation(self._next(), n)
kernel_name = 'concat_heads__softmax_full_mha__memory_aug_recurrent_mem_tr__prompt'

def setup_inputs():
    _rng = _Rng(jax.random.key(int.from_bytes(__import__("os").urandom(4), "little")))
    _w = lambda a: (lambda t: t.astype(jnp.bfloat16) if jnp.issubdtype(t.dtype, jnp.floating) else t)(jnp.asarray(a))

    def _A_setup():
        B, S, D = (1, 2048, 1024)
        return {'x': _w((lambda *s: _rng.normal(s) * 0.05)(B, S, D)), 'wqkv': _w((lambda *s: _rng.normal(s) * 0.05)(D, 3 * D)), 'wo': _w((lambda *s: _rng.normal(s) * 0.05)(D, D))}
    _A_in = _A_setup()

    def _B_setup():
        B, S, Dm = (1, 2048, 1024)
        H, Dh = (32, 128)
        M, seg = (8, 32)
        seg = min(seg, S)
        S = S // seg * seg
        return {'x': _w((lambda *s: _rng.normal(s) * 0.05)(B, S, Dm)), 'mem0': _w((lambda *s: _rng.normal(s) * 0.05)(B, M, Dm)), 'Wq': _w((lambda *s: _rng.normal(s) * 0.05)(Dm, H, Dh) * Dm ** (-0.5)), 'Wk': _w((lambda *s: _rng.normal(s) * 0.05)(Dm, H, Dh) * Dm ** (-0.5)), 'Wv': _w((lambda *s: _rng.normal(s) * 0.05)(Dm, H, Dh) * Dm ** (-0.5)), 'Wo': _w((lambda *s: _rng.normal(s) * 0.05)(H, Dh, Dm) * (H * Dh) ** (-0.5)), 'seg_len': seg}
    _B_in = _B_setup()
    return {'A_x': _A_in['x'], 'A_wqkv': _A_in['wqkv'], 'A_wo': _A_in['wo'], 'B_x': _B_in['x'], 'B_mem0': _B_in['mem0'], 'B_Wq': _B_in['Wq'], 'B_Wk': _B_in['Wk'], 'B_Wv': _B_in['Wv'], 'B_Wo': _B_in['Wo'], 'B_seg_len': _B_in['seg_len']}

def reference(A_x, A_wqkv, A_wo, B_x, B_mem0, B_Wq, B_Wk, B_Wv, B_Wo, B_seg_len):

    def _A_ref(x, wqkv, wo):
        B, S, D = x.shape
        H = 32
        Dh = D // H
        qkv = (lambda x, *d: x.transpose(*d))((x @ wqkv).reshape(B, S, 3, H, Dh), 2, 0, 3, 1, 4)
        q, k, v = (qkv[0], qkv[1], qkv[2])
        scale = Dh ** (-0.5)
        scores = jnp.einsum('bhqd,bhkd->bhqk', q, k) * scale
        p = _softmax(scores, axis=-1)
        o = jnp.einsum('bhqk,bhkd->bhqd', p, v)
        return (lambda x, *d: x.transpose(*d))(o, 0, 2, 1, 3).reshape(B, S, D) @ wo

    def _B_ref(x, mem0, Wq, Wk, Wv, Wo, seg_len):
        B, S, Dm = x.shape
        H, Dh = (Wq.shape[1], Wq.shape[2])
        M = mem0.shape[1]
        scale = Dh ** (-0.5)
        n_seg = S // seg_len
        L = M + seg_len
        idx = jnp.arange(L)
        mask = (idx[:, None] < M) | (idx[:, None] >= idx[None, :])
        mem = mem0
        outs = []
        for s in range(n_seg):
            xs = x[:, s * seg_len:(s + 1) * seg_len, :].copy()
            h = jnp.concatenate([mem, xs], axis=1)
            q = jnp.einsum('btd,dhe->bhte', h, Wq)
            k = jnp.einsum('btd,dhe->bhte', h, Wk)
            v = jnp.einsum('btd,dhe->bhte', h, Wv)
            scores = jnp.einsum('bhqe,bhke->bhqk', q, k) * scale
            scores = jnp.where(mask[None, None], scores, -1000000000.0)
            p = _softmax(scores, axis=-1)
            o = jnp.einsum('bhqk,bhke->bhqe', p, v)
            o = jnp.einsum('bhte,hed->btd', o, Wo)
            mem = o[:, :M, :].copy()
            outs.append(o[:, M:, :])
        return jnp.concatenate(outs, axis=1)
    a = _A_ref(A_x, A_wqkv, A_wo)
    b = _B_ref(B_x, B_mem0, B_Wq, B_Wk, B_Wv, B_Wo, B_seg_len)
    return jnp.concatenate([a, b], axis=-1)
```

```python
import functools
import math

import jax
import jax.numpy as jnp
from jax import lax
from jax.experimental import pallas as pl
from jax.experimental.pallas import tpu as pltpu

f32 = jnp.float32
bf16 = jnp.bfloat16
NN = (((1,), (0,)), ((), ()))
NT = (((1,), (1,)), ((), ()))
TN = (((0,), (0,)), ((), ()))
LOG2E = 1.4426950408889634


def _dot(a, b, dn=NN):
    return lax.dot_general(a, b, dn, preferred_element_type=f32)


def _kernel(ax_hbm, wqkv_hbm, awo_hbm, bx_hbm, mem0_hbm, wq_hbm, wk_hbm, wv_hbm, bwo_hbm,
            out_hbm,
            xa, wqkv, awo, qt, kk, vt, ot, lbuf, mbuf, qm0, qm1, stage_a,
            xb, mem0v, wraw, wqt, wkt, wvt, bwo, hcat, stage_b, sems,
            *, cfg):
    S, D, HA, DA = 2048, 1024, 32, 32
    HB, DB, M, SEG = 32, 128, 8, 32
    L = M + SEG
    NSEG = S // SEG
    NQ, KC, SK, UN = cfg["NQ"], cfg["KC"], cfg["SK"], cfg["UN"]

    def cp(i, src, dst):
        return pltpu.make_async_copy(src, dst, sems.at[i])
    c_ax = cp(0, ax_hbm, xa)
    c_wqkv = cp(1, wqkv_hbm, wqkv)
    c_awo = cp(2, awo_hbm, awo)
    c_wq = cp(3, wq_hbm, wraw.at[0])
    c_wk = cp(4, wk_hbm, wraw.at[1])
    c_wv = cp(5, wv_hbm, wraw.at[2])
    c_bwo = cp(6, bwo_hbm, bwo)
    c_bx = cp(7, bx_hbm, xb)
    c_mem = cp(8, mem0_hbm, mem0v)
    c_oa = cp(9, stage_a, out_hbm.at[:, 0:D])
    c_ob = cp(10, stage_b, out_hbm.at[:, D:2 * D])
    for c in (c_ax, c_wqkv, c_awo, c_wq, c_wk, c_wv, c_bwo, c_bx, c_mem):
        c.start()
    c_ax.wait()
    c_wqkv.wait()

    qscale = (DA ** -0.5) * LOG2E
    RB = cfg["RB"]

    def proj_body(rb, carry):
        r0 = pl.multiple_of(rb * RB, RB)
        x = xa[pl.ds(r0, RB), :]
        q = (_dot(x, wqkv[:, 0:D]) * qscale).astype(bf16)
        for g in range(8):
            qg = q[:, g * 128:(g + 1) * 128].T
            qt[g, :, pl.ds(r0, RB)] = qg
            qf = qg.astype(f32)
            q2 = (qf * qf).reshape(4, 4, 8, RB).sum(axis=1)
            lbuf[g * 4:(g + 1) * 4, :, pl.ds(r0, RB)] = q2
        k = _dot(x, wqkv[:, D:2 * D]).astype(bf16)
        for g in range(8):
            kg = k[:, g * 128:(g + 1) * 128]
            kk[g, pl.ds(r0, RB), :] = kg
            kf = kg.T.astype(f32)
            k2 = (kf * kf).reshape(4, 4, 8, RB).sum(axis=1)
            mbuf[g * 4:(g + 1) * 4, :, pl.ds(r0, RB)] = k2
        v = _dot(x, wqkv[:, 2 * D:3 * D]).astype(bf16)
        for g in range(8):
            vt[g * 128:(g + 1) * 128, pl.ds(r0, RB)] = v[:, g * 128:(g + 1) * 128].T
        return carry
    lax.fori_loop(0, S // RB, proj_body, 0)

    def bound_body(h, carry):
        k2 = jnp.sum(mbuf[h], axis=0, keepdims=True)
        kmax2 = jnp.max(k2, axis=1, keepdims=True)
        q2 = jnp.sum(lbuf[h], axis=0, keepdims=True)
        bound = jnp.sqrt(q2 * kmax2) * 1.001
        mbuf[h] = jnp.broadcast_to(bound, (8, S))
        return carry
    lax.fori_loop(0, HA, bound_body, 0)

    NB = S // NQ
    NIT = HA * NB
    NKC = S // KC
    rowj = lax.broadcasted_iota(jnp.int32, (128, NQ), 0) // DA

    def setup_q(i, qm_ref):
        h = i // NB
        qb = i % NB
        g = h // 4
        j = h % 4
        q0 = pl.multiple_of(qb * NQ, NQ)
        qv = qt[g, :, pl.ds(q0, NQ)]
        qm_ref[...] = jnp.where(rowj == j, qv, jnp.zeros_like(qv))
        return g

    def attn_body(ii, carry):
        gs, hs, q0s, ms = [], [], [], []
        for u in range(UN):
            i = UN * ii + u
            h = i // NB
            q0 = pl.multiple_of((i % NB) * NQ, NQ)
            hs.append(h)
            q0s.append(q0)
            gs.append(setup_q(i, (qm0, qm1)[u % 2]))
            ms.append(mbuf[h, :, pl.ds(q0, NQ)])
        l8 = [None] * UN
        o = [None] * UN
        pst = {}
        for t in range(UN * NKC + SK):
            if t < UN * NKC:
                u, kc = divmod(t, NKC)
                s = _dot(kk[gs[u], kc * KC:(kc + 1) * KC, :], (qm0, qm1)[u % 2][...])
                p = jnp.exp2(s.reshape(KC // 8, 8, NQ) - ms[u][None])
                ps = jnp.sum(p, axis=0)
                l8[u] = ps if l8[u] is None else l8[u] + ps
                pst[t] = p.reshape(KC, NQ).astype(bf16)
            tt = t - SK
            if tt >= 0:
                u, kc = divmod(tt, NKC)
                v_c = vt[pl.ds(pl.multiple_of(hs[u] * DA, DA), DA), kc * KC:(kc + 1) * KC]
                oc = _dot(v_c, pst.pop(tt))
                o[u] = oc if o[u] is None else o[u] + oc
                if kc == NKC - 1:
                    l = jnp.sum(l8[u], axis=0, keepdims=True)
                    lbuf[hs[u], :, pl.ds(q0s[u], NQ)] = jnp.broadcast_to(l, (8, NQ))
                    ot[pl.ds(pl.multiple_of(hs[u] * DA, DA), DA), pl.ds(q0s[u], NQ)] = (o[u] * (1.0 / l)).astype(bf16)
        return carry
    lax.fori_loop(0, NIT // UN, attn_body, 0)

    def check_body(h, carry):
        lv = lbuf[h]
        bad = jnp.logical_not(jnp.logical_and(lv > 2.0 ** -80, lv < 2.0 ** 80))
        nbad = jnp.sum(bad.astype(jnp.int32))

        @pl.when(nbad != 0)
        def _():
            def fb_body(qb, c2):
                q0 = pl.multiple_of(qb * NQ, NQ)
                g = setup_q(h * NB + qb, qm0)
                s = _dot(kk[g], qm0[...])
                m = jnp.max(s, axis=0, keepdims=True)
                p = jnp.exp2(s - m)
                l = jnp.sum(p, axis=0, keepdims=True)
                hrow = pl.ds(pl.multiple_of(h * DA, DA), DA)
                oo = _dot(vt[hrow, :], p.astype(bf16))
                ot[hrow, pl.ds(q0, NQ)] = (oo * (1.0 / l)).astype(bf16)
                return c2
            lax.fori_loop(0, NB, fb_body, 0)
        return carry
    lax.fori_loop(0, HA, check_body, 0)

    c_awo.wait()

    def oproj_body(rb, carry):
        r0 = pl.multiple_of(rb * RB, RB)
        o_blk = ot[:, pl.ds(r0, RB)]
        stage_a[pl.ds(r0, RB), :] = _dot(o_blk, awo[...], TN).astype(bf16)
        return carry
    lax.fori_loop(0, S // RB, oproj_body, 0)
    c_oa.start()

    c_wq.wait()
    c_wk.wait()
    c_wv.wait()

    def relayout_body(dc, carry):
        for w, dst in enumerate((wqt, wkt, wvt)):
            for sub in range(2):
                d0 = pl.multiple_of(dc * 32 + sub * 16, 16)
                dst[:, pl.ds(d0, 16), :] = jnp.swapaxes(wraw[w, pl.ds(d0, 16)], 0, 1)
        return carry
    lax.fori_loop(0, D // 32, relayout_body, 0)
    c_bwo.wait()
    c_bx.wait()
    c_mem.wait()

    bscale = DB ** -0.5
    row = lax.broadcasted_iota(jnp.int32, (L, L), 0)
    col = lax.broadcasted_iota(jnp.int32, (L, L), 1)
    mask = (row < M) | (row >= col)
    hcat[0:M, :] = mem0v[...].astype(f32)
    order = cfg["order"]

    def seg_body(s, carry):
        r0 = pl.multiple_of(s * SEG, SEG)
        hcat[M:L, :] = xb[pl.ds(r0, SEG), :].astype(f32)
        hc = hcat[...]
        st = {}
        acc = [None]

        def Q(h): st['q', h] = _dot(hc, wqt[h])
        def K(h): st['k', h] = _dot(hc, wkt[h])
        def V(h): st['v', h] = _dot(hc, wvt[h])

        def SC(h):
            sc = _dot(st.pop(('q', h)), st.pop(('k', h)).astype(bf16), NT) * bscale
            sc = jnp.where(mask, sc, -1e9)
            m = jnp.max(sc, axis=-1, keepdims=True)
            p = jnp.exp(sc - m)
            l = jnp.sum(p, axis=-1, keepdims=True)
            st['p', h] = p
            st['rl', h] = 1.0 / l

        def PV(h):
            oo = _dot(st.pop(('p', h)), st.pop(('v', h)).astype(bf16))
            st['o', h] = oo * st.pop(('rl', h))

        def O(h):
            po = _dot(st.pop(('o', h)), bwo[h])
            acc[0] = po if acc[0] is None else acc[0] + po
        fns = dict(Q=Q, K=K, V=V, SC=SC, PV=PV, O=O)
        for name, h in order:
            fns[name](h)
        accb = acc[0].astype(bf16)
        hcat[0:M, :] = accb[0:M].astype(f32)
        stage_b[pl.ds(r0, SEG), :] = accb[M:L]
        return carry
    lax.fori_loop(0, NSEG, seg_body, 0)
    c_ob.start()
    c_oa.wait()
    c_ob.wait()


def _b_order(dq=(('Q', 0), ('K', 0), ('V', 0), ('SC', -1), ('PV', -2), ('O', -3)), H=32):
    out = []
    for i in range(H + 8):
        for name, off in dq:
            h = i + off
            if 0 <= h < H:
                out.append((name, h))
    return tuple(out)


CFG = dict(NQ=512, KC=128, SK=2, UN=2, RB=256, order=_b_order())


@functools.partial(jax.jit, static_argnames=("B_seg_len",))
def pallas_concat_heads__softmax_full_mha__memory_aug_recurrent_mem_tr__prompt_kernel(
        A_x, A_wqkv, A_wo, B_x, B_mem0, B_Wq, B_Wk, B_Wv, B_Wo, B_seg_len):
    S, D = 2048, 1024
    assert B_seg_len == 32
    any_ = pl.BlockSpec(memory_space=pl.ANY)
    V = pltpu.VMEM
    cfg = CFG
    NQ = cfg["NQ"]
    scratch = [
        V((S, D), bf16), V((D, 3 * D), bf16), V((D, D), bf16),
        V((8, 128, S), bf16), V((8, S, 128), bf16), V((D, S), bf16), V((D, S), bf16),
        V((32, 8, S), f32), V((32, 8, S), f32),
        V((128, NQ), bf16), V((128, NQ), bf16), V((S, D), bf16),
        V((S, D), bf16), V((8, D), bf16), V((3, D, 32, 128), bf16),
        V((32, D, 128), bf16), V((32, D, 128), bf16), V((32, D, 128), bf16),
        V((32, 128, D), bf16), V((40, D), f32), V((S, D), bf16),
        pltpu.SemaphoreType.DMA((11,)),
    ]
    out = pl.pallas_call(
        functools.partial(_kernel, cfg=cfg),
        out_shape=jax.ShapeDtypeStruct((S, 2 * D), bf16),
        in_specs=[any_] * 9,
        out_specs=any_,
        scratch_shapes=scratch,
        compiler_params=pltpu.CompilerParams(vmem_limit_bytes=124 * 2 ** 20),
    )(A_x.reshape(S, D), A_wqkv, A_wo, B_x.reshape(S, D), B_mem0.reshape(8, D), B_Wq, B_Wk, B_Wv, B_Wo)
    return out.reshape(1, S, 2 * D)
```

```python
import functools

import jax
import jax.numpy as jnp
from jax import lax
from jax.experimental import pallas as pl
from jax.experimental.pallas import tpu as pltpu

f32 = jnp.float32
bf16 = jnp.bfloat16
NN = (((1,), (0,)), ((), ()))
NT = (((1,), (1,)), ((), ()))
TN = (((0,), (0,)), ((), ()))
LOG2E = 1.4426950408889634

S, D, HA, DA = 2048, 1024, 32, 32
HB, DB, M, SEG = 32, 128, 8, 32
L = M + SEG
NSEG = S // SEG


def _dot(a, b, dn=NN):
    return lax.dot_general(a, b, dn, preferred_element_type=f32)


def _kernel(ax_hbm, wqkv_hbm, awo_hbm, bx_hbm, mem0_hbm, wq_hbm, wk_hbm, wv_hbm, bwo_hbm,
            out_hbm,
            xa, wqkv, awo, qt, kk, wt, vt, ot, q2buf, kmpart, kmx, lbuf, qm, stage_a,
            xb, mem0v, wraw, bwo, hcat, stage_b, xsems, sems,
            *, cfg):
    NQ, KC, SK, UN, RB = cfg["NQ"], cfg["KC"], cfg["SK"], cfg["UN"], cfg["RB"]
    NRB = S // RB

    def cp(i, src, dst):
        return pltpu.make_async_copy(src, dst, sems.at[i])

    def cx(rb):
        return pltpu.make_async_copy(ax_hbm.at[pl.ds(rb * RB, RB), :], xa.at[pl.ds(rb * RB, RB), :], xsems.at[rb])
    c_w = [cp(i, wqkv_hbm.at[:, i * D:(i + 1) * D], wqkv.at[i]) for i in range(3)]
    c_wq = cp(3, wq_hbm, wraw.at[0])
    c_wk = cp(4, wk_hbm, wraw.at[1])
    c_wv = cp(5, wv_hbm, wraw.at[2])
    c_awo = cp(6, awo_hbm, awo)
    c_bwo = cp(7, bwo_hbm, bwo)
    c_bx = cp(8, bx_hbm, xb)
    c_mem = cp(9, mem0_hbm, mem0v)
    c_oa = cp(10, stage_a, out_hbm.at[:, 0:D])
    c_w[0].start()
    cx(0).start()
    for rb in range(1, NRB):
        cx(rb).start()
    c_w[1].start()
    c_w[2].start()

    qscale = (DA ** -0.5) * LOG2E
    c_w[0].wait()

    def q_body(rb, carry):
        cx(rb).wait()
        r0 = pl.multiple_of(rb * RB, RB)
        q = (_dot(xa[pl.ds(r0, RB), :], wqkv[0]) * qscale).astype(bf16)
        for g in range(8):
            qg = q[:, g * 128:(g + 1) * 128].T
            qt[g, :, pl.ds(r0, RB)] = qg
            qf = qg.astype(f32)
            q2buf[g * 4:(g + 1) * 4, pl.ds(r0, RB)] = jnp.sum((qf * qf).reshape(4, DA, RB), axis=1)
        return carry
    lax.fori_loop(0, NRB, q_body, 0)

    for c in (c_wq, c_wk, c_wv, c_awo, c_bwo, c_bx, c_mem):
        c.start()
    c_w[1].wait()

    def k_body(rb, carry):
        r0 = pl.multiple_of(rb * RB, RB)
        k = _dot(xa[pl.ds(r0, RB), :], wqkv[1]).astype(bf16)
        for g in range(8):
            kg = k[:, g * 128:(g + 1) * 128]
            kk[g, pl.ds(r0, RB), :] = kg
            kf = kg.T.astype(f32)
            k2 = jnp.sum((kf * kf).reshape(4, DA, RB), axis=1)
            km = k2[:, 0:128]
            for t in range(1, RB // 128):
                km = jnp.maximum(km, k2[:, t * 128:(t + 1) * 128])
            kmpart[rb, g * 4:(g + 1) * 4, :] = km
        return carry
    lax.fori_loop(0, NRB, k_body, 0)

    c_w[2].wait()

    def v_body(rb, carry):
        r0 = pl.multiple_of(rb * RB, RB)
        v = _dot(xa[pl.ds(r0, RB), :], wqkv[2]).astype(bf16)
        for g in range(8):
            vt[g * 128:(g + 1) * 128, pl.ds(r0, RB)] = v[:, g * 128:(g + 1) * 128].T
        return carry
    lax.fori_loop(0, NRB, v_body, 0)

    kmx[...] = jnp.broadcast_to(jnp.max(jnp.max(kmpart[...], axis=0), axis=1, keepdims=True), (HA, 128))

    NB = S // NQ
    NIT = HA * NB
    NKC = S // KC
    NBODY = NIT // UN
    rowj = lax.broadcasted_iota(jnp.int32, (128, NQ), 0) // DA

    def kchunk(g, kc0, n):
        return kk[g, pl.ds(kc0, n), :]

    def setup_q(i, slot):
        h = i // NB
        qb = i % NB
        g = h // 4
        j = h % 4
        q0 = pl.multiple_of(qb * NQ, NQ)
        qv = qt[g, :, pl.ds(q0, NQ)]
        qm[slot] = jnp.where(rowj == j, qv, jnp.zeros_like(qv))

    c_wq.wait()
    c_wk.wait()
    c_wv.wait()
    NPIECE = 3 * (D // 16)
    PPB = NPIECE // NBODY

    def relayout_piece(pc):
        w = pc // (D // 16)
        d0 = pl.multiple_of((pc % (D // 16)) * 16, 16)
        wt[pl.ds(32 * w, 32), pl.ds(d0, 16), :] = jnp.swapaxes(wraw[w, pl.ds(d0, 16)], 0, 1)

    setup_q(0, 0)
    piece_at = cfg["piece_at"]

    def attn_body(ii, carry):
        gs, hs, q0s, ms = [], [], [], []
        for u in range(UN):
            i = UN * ii + u
            h = i // NB
            q0 = pl.multiple_of((i % NB) * NQ, NQ)
            hs.append(h)
            q0s.append(q0)
            gs.append(h // 4)
            if u > 0:
                setup_q(i, u)
            km = kmx[pl.ds(h, 1), :]
            bound = jnp.sqrt(q2buf[pl.ds(h, 1), pl.ds(q0, NQ)] * jnp.concatenate([km] * (NQ // 128), axis=1)) * 1.001
            ms.append(jnp.broadcast_to(bound, (8, NQ)))
        l8 = [None] * UN
        o = [None] * UN
        pst = {}
        npc = 0
        for t in range(UN * NKC + SK):
            if t < UN * NKC:
                u, kc = divmod(t, NKC)
                s = _dot(kchunk(gs[u], kc * KC, KC), qm[u])
                p = jnp.exp2(s.reshape(KC // 8, 8, NQ) - ms[u][None])
                ps = jnp.sum(p, axis=0)
                l8[u] = ps if l8[u] is None else l8[u] + ps
                pst[t] = p.reshape(KC, NQ).astype(bf16)
                if u == 0 and kc == NKC - 1:
                    setup_q(jnp.minimum(UN * ii + UN, NIT - 1), 0)
                if cfg['inl'] and t in piece_at:
                    relayout_piece(ii * PPB + npc)
                    npc += 1
            tt = t - SK
            if tt >= 0:
                u, kc = divmod(tt, NKC)
                hrow = pl.ds(pl.multiple_of(hs[u] * DA, DA), DA)
                oc = _dot(vt[hrow, kc * KC:(kc + 1) * KC], pst.pop(tt))
                o[u] = oc if o[u] is None else o[u] + oc
                if kc == NKC - 1:
                    l = jnp.sum(l8[u], axis=0, keepdims=True)
                    lbuf[pl.ds(hs[u], 1), pl.ds(q0s[u], NQ)] = l
                    ot[hrow, pl.ds(q0s[u], NQ)] = (o[u] * (1.0 / l)).astype(bf16)
        assert npc == PPB or not cfg['inl'], (npc, PPB)
        return carry
    lax.fori_loop(0, NBODY, attn_body, 0)

    def is_bad(lv):
        return jnp.logical_not(jnp.logical_and(lv > 2.0 ** -80, lv < 2.0 ** 80))
    nbad_all = jnp.sum(is_bad(lbuf[...]).astype(jnp.int32))

    @pl.when(nbad_all != 0)
    def _():
        def check_body(h, carry):
            nbad = jnp.sum(is_bad(lbuf[pl.ds(h, 1), :]).astype(jnp.int32))

            @pl.when(nbad != 0)
            def _():
                def fb_body(qb, c2):
                    q0 = pl.multiple_of(qb * NQ, NQ)
                    setup_q(h * NB + qb, 0)
                    g = h // 4
                    hrow = pl.ds(pl.multiple_of(h * DA, DA), DA)
                    s0 = _dot(kk[g, 0:1024], qm[0])
                    s1 = _dot(kk[g, 1024:2048], qm[0])
                    m = jnp.maximum(jnp.max(s0, axis=0, keepdims=True), jnp.max(s1, axis=0, keepdims=True))
                    p0 = jnp.exp2(s0 - m)
                    p1 = jnp.exp2(s1 - m)
                    l = jnp.sum(p0, axis=0, keepdims=True) + jnp.sum(p1, axis=0, keepdims=True)
                    oo = _dot(vt[hrow, 0:1024], p0.astype(bf16)) + _dot(vt[hrow, 1024:2048], p1.astype(bf16))
                    ot[hrow, pl.ds(q0, NQ)] = (oo * (1.0 / l)).astype(bf16)
                    return c2
                lax.fori_loop(0, NB, fb_body, 0)
            return carry
        lax.fori_loop(0, HA, check_body, 0)

    c_awo.wait()

    def oproj_body(rb, carry):
        r0 = pl.multiple_of(rb * RB, RB)
        stage_a[pl.ds(r0, RB), :] = _dot(ot[:, pl.ds(r0, RB)], awo[...], TN).astype(bf16)
        return carry
    lax.fori_loop(0, NRB, oproj_body, 0)
    c_oa.start()

    if not cfg['inl']:
        def rl_body(j, carry):
            for pp in range(6):
                relayout_piece(j * 6 + pp)
            return carry
        lax.fori_loop(0, NPIECE // 6, rl_body, 0)
    c_bwo.wait()
    c_bx.wait()
    c_mem.wait()

    bscale = DB ** -0.5
    row = lax.broadcasted_iota(jnp.int32, (L, L), 0)
    col = lax.broadcasted_iota(jnp.int32, (L, L), 1)
    mask = (row < M) | (row >= col)
    hcat[0:M, :] = mem0v[...].astype(f32)
    order = cfg["order"]

    def seg_body(s, carry):
        r0 = pl.multiple_of(s * SEG, SEG)
        hcat[M:L, :] = xb[pl.ds(r0, SEG), :].astype(f32)
        hc = hcat[...]
        st = {}
        acc = [None]

        def Q(h): st['q', h] = _dot(hc, wt[h])
        def K(h): st['k', h] = _dot(hc, wt[32 + h])
        def V(h): st['v', h] = _dot(hc, wt[64 + h])

        def SC(h):
            sc = _dot(st.pop(('q', h)), st.pop(('k', h)).astype(bf16), NT) * bscale
            sc = jnp.where(mask, sc, -1e9)
            m = jnp.max(sc, axis=-1, keepdims=True)
            p = jnp.exp(sc - m)
            l = jnp.sum(p, axis=-1, keepdims=True)
            st['p', h] = p
            st['rl', h] = 1.0 / l

        def PV(h):
            oo = _dot(st.pop(('p', h)), st.pop(('v', h)).astype(bf16))
            st['o', h] = oo * st.pop(('rl', h))

        def O(h):
            po = _dot(st.pop(('o', h)), bwo[h])
            acc[0] = po if acc[0] is None else acc[0] + po
        fns = dict(Q=Q, K=K, V=V, SC=SC, PV=PV, O=O)
        for name, h in order:
            fns[name](h)
        accb = acc[0].astype(bf16)
        hcat[0:M, :] = accb[0:M].astype(f32)
        stage_b[pl.ds(r0, SEG), :] = accb[M:L]
        return carry

    NOB = cfg["NOB"]
    SPB = NSEG // NOB
    OR = SPB * SEG

    def c_ob(blk):
        r0 = pl.multiple_of(blk * OR, OR)
        return pltpu.make_async_copy(stage_b.at[pl.ds(r0, OR), :], out_hbm.at[pl.ds(r0, OR), D:2 * D], sems.at[11])

    def blk_body(blk, carry):
        lax.fori_loop(blk * SPB, (blk + 1) * SPB, seg_body, 0)
        c_ob(blk).start()
        return carry
    lax.fori_loop(0, NOB, blk_body, 0)
    c_oa.wait()
    for blk in range(NOB):
        c_ob(blk).wait()


def _tail_order(d_o=6, ntail=(2, 4)):
    dq = [('Q', 0), ('K', 0), ('V', 0), ('SC', -1), ('PV', -2), ('O', -d_o)]
    out = []
    for i in range(HB):
        for name, off in dq:
            h = i + off
            if 0 <= h < HB:
                out.append((name, h))
    done = set(out)
    os_ = [('O', h) for h in range(HB) if ('O', h) not in done]
    t = [('SC', HB - 1)] + os_[:ntail[0]] + [('PV', HB - 2)] + os_[ntail[0]:ntail[1]] + [('PV', HB - 1)] + os_[ntail[1]:]
    return tuple(out + t)


CFG = dict(inl=False, NQ=512, KC=256, SK=1, UN=4, RB=512, NOB=8, order=_tail_order(), piece_at=(2, 7, 12, 17, 22, 27))


@functools.partial(jax.jit, static_argnames=("B_seg_len",))
def pallas_concat_heads__softmax_full_mha__memory_aug_recurrent_mem_tr__prompt_kernel(
        A_x, A_wqkv, A_wo, B_x, B_mem0, B_Wq, B_Wk, B_Wv, B_Wo, B_seg_len):
    assert B_seg_len == SEG
    any_ = pl.BlockSpec(memory_space=pl.ANY)
    V = pltpu.VMEM
    cfg = CFG
    NQ, UN, RB = cfg["NQ"], cfg["UN"], cfg["RB"]
    scratch = [
        V((S, D), bf16), V((3, D, D), bf16), V((D, D), bf16),
        V((8, 128, S), bf16), V((8, S, 128), bf16), V((96, 1024, 128), bf16), V((D, S), bf16), V((D, S), bf16),
        V((HA, S), f32), V((S // RB, HA, 128), f32), V((HA, 128), f32), V((HA, S), f32),
        V((UN, 128, NQ), bf16), V((S, D), bf16),
        V((S, D), bf16), V((8, D), bf16), V((3, D, 32, 128), bf16),
        V((32, 128, D), bf16), V((L, D), f32), V((S, D), bf16),
        pltpu.SemaphoreType.DMA((S // RB,)),
        pltpu.SemaphoreType.DMA((12,)),
    ]
    out = pl.pallas_call(
        functools.partial(_kernel, cfg=cfg),
        out_shape=jax.ShapeDtypeStruct((S, 2 * D), bf16),
        in_specs=[any_] * 9,
        out_specs=any_,
        scratch_shapes=scratch,
        compiler_params=pltpu.CompilerParams(vmem_limit_bytes=124 * 2 ** 20),
    )(A_x.reshape(S, D), A_wqkv, A_wo, B_x.reshape(S, D), B_mem0.reshape(8, D), B_Wq, B_Wk, B_Wv, B_Wo)
    return out.reshape(1, S, 2 * D)
```

```python
import functools

import jax
import jax.numpy as jnp
from jax import lax
from jax.experimental import pallas as pl
from jax.experimental.pallas import tpu as pltpu

f32 = jnp.float32
bf16 = jnp.bfloat16
NN = (((1,), (0,)), ((), ()))
NT = (((1,), (1,)), ((), ()))
TN = (((0,), (0,)), ((), ()))
LOG2E = 1.4426950408889634

S, D, HA, DA = 2048, 1024, 32, 32
HB, DB, M, SEG = 32, 128, 8, 32
L = M + SEG
NSEG = S // SEG


def _dot(a, b, dn=NN):
    return lax.dot_general(a, b, dn, preferred_element_type=f32)


def _kernel(ax_hbm, wqkv_hbm, awo_hbm, bx_hbm, mem0_hbm, wq_hbm, wk_hbm, wv_hbm, bwo_hbm,
            out_hbm,
            xa, wqkv, awo, qt, kk, vt, ot, q2buf, kmpart, kmx, lbuf, qm, stage_a,
            xb, mem0v, uw, bwo, hcat, stage_b, xsems, sems,
            *, cfg):
    NQ, KC, SK, UN, RB = cfg["NQ"], cfg["KC"], cfg["SK"], cfg["UN"], cfg["RB"]
    NRB = S // RB

    def cp(i, src, dst):
        return pltpu.make_async_copy(src, dst, sems.at[i])

    def cx(rb):
        return pltpu.make_async_copy(ax_hbm.at[pl.ds(rb * RB, RB), :], xa.at[pl.ds(rb * RB, RB), :], xsems.at[rb])
    c_w = [cp(i, wqkv_hbm.at[:, i * D:(i + 1) * D], wqkv.at[i]) for i in range(3)]
    c_bw = []
    for w, src in enumerate((wq_hbm, wk_hbm, wv_hbm)):
        su = src.bitcast(jnp.uint32)
        c_bw.append([cp(3 + w, su.at[:, hp, :], uw.at[w, hp]) for hp in range(HB // 2)])
    c_awo = cp(6, awo_hbm, awo)
    c_bwo = cp(7, bwo_hbm, bwo)
    c_bx = cp(8, bx_hbm, xb)
    c_mem = cp(9, mem0_hbm, mem0v)
    c_oa = cp(10, stage_a, out_hbm.at[:, 0:D])
    c_w[0].start()
    cx(0).start()
    for rb in range(1, NRB):
        cx(rb).start()
    c_w[1].start()
    c_w[2].start()

    qscale = (DA ** -0.5) * LOG2E
    c_w[0].wait()

    def q_body(rb, carry):
        cx(rb).wait()
        r0 = pl.multiple_of(rb * RB, RB)
        q = (_dot(xa[pl.ds(r0, RB), :], wqkv[0]) * qscale).astype(bf16)
        for g in range(8):
            qg = q[:, g * 128:(g + 1) * 128].T
            qt[g, :, pl.ds(r0, RB)] = qg
            qf = qg.astype(f32)
            q2buf[g * 4:(g + 1) * 4, pl.ds(r0, RB)] = jnp.sum((qf * qf).reshape(4, DA, RB), axis=1)
        return carry
    lax.fori_loop(0, NRB, q_body, 0)

    for cs in c_bw:
        for c in cs:
            c.start()
    for c in (c_awo, c_bwo, c_bx, c_mem):
        c.start()
    c_w[1].wait()

    def k_body(rb, carry):
        r0 = pl.multiple_of(rb * RB, RB)
        k = _dot(xa[pl.ds(r0, RB), :], wqkv[1]).astype(bf16)
        for g in range(8):
            kg = k[:, g * 128:(g + 1) * 128]
            kk[g, pl.ds(r0, RB), :] = kg
            kf = kg.T.astype(f32)
            k2 = jnp.sum((kf * kf).reshape(4, DA, RB), axis=1)
            km = k2[:, 0:128]
            for t in range(1, RB // 128):
                km = jnp.maximum(km, k2[:, t * 128:(t + 1) * 128])
            kmpart[rb, g * 4:(g + 1) * 4, :] = km
        return carry
    lax.fori_loop(0, NRB, k_body, 0)

    c_w[2].wait()

    def v_body(rb, carry):
        r0 = pl.multiple_of(rb * RB, RB)
        v = _dot(xa[pl.ds(r0, RB), :], wqkv[2]).astype(bf16)
        for g in range(8):
            vt[g * 128:(g + 1) * 128, pl.ds(r0, RB)] = v[:, g * 128:(g + 1) * 128].T
        return carry
    lax.fori_loop(0, NRB, v_body, 0)

    kmx[...] = jnp.broadcast_to(jnp.max(jnp.max(kmpart[...], axis=0), axis=1, keepdims=True), (HA, 128))

    NB = S // NQ
    NIT = HA * NB
    NKC = S // KC
    NBODY = NIT // UN
    rowj = lax.broadcasted_iota(jnp.int32, (128, NQ), 0) // DA

    def kchunk(g, kc0, n):
        return kk[g, pl.ds(kc0, n), :]

    def setup_q(i, slot):
        h = i // NB
        qb = i % NB
        g = h // 4
        j = h % 4
        q0 = pl.multiple_of(qb * NQ, NQ)
        qv = qt[g, :, pl.ds(q0, NQ)]
        qm[slot] = jnp.where(rowj == j, qv, jnp.zeros_like(qv))

    setup_q(0, 0)

    def attn_body(ii, carry):
        gs, hs, q0s, ms = [], [], [], []
        for u in range(UN):
            i = UN * ii + u
            h = i // NB
            q0 = pl.multiple_of((i % NB) * NQ, NQ)
            hs.append(h)
            q0s.append(q0)
            gs.append(h // 4)
            if u > 0:
                setup_q(i, u)
            km = kmx[pl.ds(h, 1), :]
            bound = jnp.sqrt(q2buf[pl.ds(h, 1), pl.ds(q0, NQ)] * jnp.concatenate([km] * (NQ // 128), axis=1)) * 1.001
            ms.append(jnp.broadcast_to(bound, (8, NQ)))
        l8 = [None] * UN
        o = [None] * UN
        pst = {}
        for t in range(UN * NKC + SK):
            if t < UN * NKC:
                u, kc = divmod(t, NKC)
                s = _dot(kchunk(gs[u], kc * KC, KC), qm[u])
                p = jnp.exp2(s.reshape(KC // 8, 8, NQ) - ms[u][None])
                ps = jnp.sum(p, axis=0)
                l8[u] = ps if l8[u] is None else l8[u] + ps
                pst[t] = p.reshape(KC, NQ).astype(bf16)
                if u == 0 and kc == NKC - 1:
                    setup_q(jnp.minimum(UN * ii + UN, NIT - 1), 0)
            tt = t - SK
            if tt >= 0:
                u, kc = divmod(tt, NKC)
                hrow = pl.ds(pl.multiple_of(hs[u] * DA, DA), DA)
                oc = _dot(vt[hrow, kc * KC:(kc + 1) * KC], pst.pop(tt))
                o[u] = oc if o[u] is None else o[u] + oc
                if kc == NKC - 1:
                    l = jnp.sum(l8[u], axis=0, keepdims=True)
                    lbuf[pl.ds(hs[u], 1), pl.ds(q0s[u], NQ)] = l
                    ot[hrow, pl.ds(q0s[u], NQ)] = (o[u] * (1.0 / l)).astype(bf16)
        return carry
    lax.fori_loop(0, NBODY, attn_body, 0)

    def is_bad(lv):
        return jnp.logical_not(jnp.logical_and(lv > 2.0 ** -80, lv < 2.0 ** 80))
    nbad_all = jnp.sum(is_bad(lbuf[...]).astype(jnp.int32))

    @pl.when(nbad_all != 0)
    def _():
        def check_body(h, carry):
            nbad = jnp.sum(is_bad(lbuf[pl.ds(h, 1), :]).astype(jnp.int32))

            @pl.when(nbad != 0)
            def _():
                def fb_body(qb, c2):
                    q0 = pl.multiple_of(qb * NQ, NQ)
                    setup_q(h * NB + qb, 0)
                    g = h // 4
                    hrow = pl.ds(pl.multiple_of(h * DA, DA), DA)
                    s0 = _dot(kk[g, 0:1024], qm[0])
                    s1 = _dot(kk[g, 1024:2048], qm[0])
                    m = jnp.maximum(jnp.max(s0, axis=0, keepdims=True), jnp.max(s1, axis=0, keepdims=True))
                    p0 = jnp.exp2(s0 - m)
                    p1 = jnp.exp2(s1 - m)
                    l = jnp.sum(p0, axis=0, keepdims=True) + jnp.sum(p1, axis=0, keepdims=True)
                    oo = _dot(vt[hrow, 0:1024], p0.astype(bf16)) + _dot(vt[hrow, 1024:2048], p1.astype(bf16))
                    ot[hrow, pl.ds(q0, NQ)] = (oo * (1.0 / l)).astype(bf16)
                    return c2
                lax.fori_loop(0, NB, fb_body, 0)
            return carry
        lax.fori_loop(0, HA, check_body, 0)

    c_awo.wait()

    def oproj_body(rb, carry):
        r0 = pl.multiple_of(rb * RB, RB)
        stage_a[pl.ds(r0, RB), :] = _dot(ot[:, pl.ds(r0, RB)], awo[...], TN).astype(bf16)
        return carry
    lax.fori_loop(0, NRB, oproj_body, 0)
    c_oa.start()

    for cs in c_bw:
        for c in cs:
            c.wait()
    c_bwo.wait()
    c_bx.wait()
    c_mem.wait()

    bscale = DB ** -0.5
    row = lax.broadcasted_iota(jnp.int32, (L, L), 0)
    col = lax.broadcasted_iota(jnp.int32, (L, L), 1)
    mask = (row < M) | (row >= col)
    hcat[0:M, :] = mem0v[...].astype(f32)
    order = cfg["order"]

    def bw(w, h):
        x = uw[w, h // 2]
        if h % 2:
            x = x >> 16
        return pltpu.bitcast(x.astype(jnp.uint16), bf16)

    def seg_body(s, carry):
        r0 = pl.multiple_of(s * SEG, SEG)
        hcat[M:L, :] = xb[pl.ds(r0, SEG), :].astype(f32)
        hc = hcat[...]
        st = {}
        acc = [None]

        def Q(h): st['q', h] = _dot(hc, bw(0, h))
        def K(h): st['k', h] = _dot(hc, bw(1, h))
        def V(h): st['v', h] = _dot(hc, bw(2, h))

        def SC(h):
            sc = _dot(st.pop(('q', h)), st.pop(('k', h)).astype(bf16), NT) * bscale
            sc = jnp.where(mask, sc, -1e9)
            m = jnp.max(sc, axis=-1, keepdims=True)
            p = jnp.exp(sc - m)
            l = jnp.sum(p, axis=-1, keepdims=True)
            st['p', h] = p
            st['rl', h] = 1.0 / l

        def PV(h):
            oo = _dot(st.pop(('p', h)), st.pop(('v', h)).astype(bf16))
            st['o', h] = oo * st.pop(('rl', h))

        def O(h):
            po = _dot(st.pop(('o', h)), bwo[h])
            acc[0] = po if acc[0] is None else acc[0] + po
        fns = dict(Q=Q, K=K, V=V, SC=SC, PV=PV, O=O)
        for name, h in order:
            fns[name](h)
        accb = acc[0].astype(bf16)
        hcat[0:M, :] = accb[0:M].astype(f32)
        stage_b[pl.ds(r0, SEG), :] = accb[M:L]
        return carry

    NOB = cfg["NOB"]
    SPB = NSEG // NOB
    OR = SPB * SEG

    def c_ob(blk):
        r0 = pl.multiple_of(blk * OR, OR)
        return pltpu.make_async_copy(stage_b.at[pl.ds(r0, OR), :], out_hbm.at[pl.ds(r0, OR), D:2 * D], sems.at[11])

    def blk_body(blk, carry):
        lax.fori_loop(blk * SPB, (blk + 1) * SPB, seg_body, 0)
        c_ob(blk).start()
        return carry
    lax.fori_loop(0, NOB, blk_body, 0)
    c_oa.wait()
    for blk in range(NOB):
        c_ob(blk).wait()


def _tail_order(d_o=6, ntail=(2, 4)):
    dq = [('Q', 0), ('K', 0), ('V', 0), ('SC', -1), ('PV', -2), ('O', -d_o)]
    out = []
    for i in range(HB):
        for name, off in dq:
            h = i + off
            if 0 <= h < HB:
                out.append((name, h))
    done = set(out)
    os_ = [('O', h) for h in range(HB) if ('O', h) not in done]
    t = [('SC', HB - 1)] + os_[:ntail[0]] + [('PV', HB - 2)] + os_[ntail[0]:ntail[1]] + [('PV', HB - 1)] + os_[ntail[1]:]
    return tuple(out + t)


CFG = dict(NQ=512, KC=256, SK=1, UN=4, RB=512, NOB=8, order=_tail_order())


@functools.partial(jax.jit, static_argnames=("B_seg_len",))
def pallas_concat_heads__softmax_full_mha__memory_aug_recurrent_mem_tr__prompt_kernel(
        A_x, A_wqkv, A_wo, B_x, B_mem0, B_Wq, B_Wk, B_Wv, B_Wo, B_seg_len):
    assert B_seg_len == SEG
    any_ = pl.BlockSpec(memory_space=pl.ANY)
    V = pltpu.VMEM
    cfg = CFG
    NQ, UN, RB = cfg["NQ"], cfg["UN"], cfg["RB"]
    scratch = [
        V((S, D), bf16), V((3, D, D), bf16), V((D, D), bf16),
        V((8, 128, S), bf16), V((8, S, 128), bf16), V((D, S), bf16), V((D, S), bf16),
        V((HA, S), f32), V((S // RB, HA, 128), f32), V((HA, 128), f32), V((HA, S), f32),
        V((UN, 128, NQ), bf16), V((S, D), bf16),
        V((S, D), bf16), V((8, D), bf16), V((3, HB // 2, D, DB), jnp.uint32),
        V((32, 128, D), bf16), V((L, D), f32), V((S, D), bf16),
        pltpu.SemaphoreType.DMA((S // RB,)),
        pltpu.SemaphoreType.DMA((12,)),
    ]
    out = pl.pallas_call(
        functools.partial(_kernel, cfg=cfg),
        out_shape=jax.ShapeDtypeStruct((S, 2 * D), bf16),
        in_specs=[any_] * 9,
        out_specs=any_,
        scratch_shapes=scratch,
        compiler_params=pltpu.CompilerParams(vmem_limit_bytes=124 * 2 ** 20),
    )(A_x.reshape(S, D), A_wqkv, A_wo, B_x.reshape(S, D), B_mem0.reshape(8, D), B_Wq, B_Wk, B_Wv, B_Wo)
    return out.reshape(1, S, 2 * D)
```

```python
import functools

import jax
import jax.numpy as jnp
from jax import lax
from jax.experimental import pallas as pl
from jax.experimental.pallas import tpu as pltpu

f32 = jnp.float32
bf16 = jnp.bfloat16
NN = (((1,), (0,)), ((), ()))
NT = (((1,), (1,)), ((), ()))
TN = (((0,), (0,)), ((), ()))
LOG2E = 1.4426950408889634

S, D, HA, DA = 2048, 1024, 32, 32
HB, DB, M, SEG = 32, 128, 8, 32
L = M + SEG
NSEG = S // SEG


def _dot(a, b, dn=NN):
    return lax.dot_general(a, b, dn, preferred_element_type=f32)


def _kernel(ax_hbm, wqkv_hbm, awo_hbm, bx_hbm, mem0_hbm, wq_hbm, wk_hbm, wv_hbm, bwo_hbm,
            out_hbm,
            xa, wqkv, awo, qt, kk, vt, ot, q2buf, kmpart, kmx, lbuf, qm, stage_a,
            xb, mem0v, uw, bwo, hcat, stage_b, xsems, sems,
            *, cfg):
    NQ, KC, SK, UN, RB = cfg["NQ"], cfg["KC"], cfg["SK"], cfg["UN"], cfg["RB"]
    NRB = S // RB

    def cp(i, src, dst):
        return pltpu.make_async_copy(src, dst, sems.at[i])

    def cx(rb):
        return pltpu.make_async_copy(ax_hbm.at[pl.ds(rb * RB, RB), :], xa.at[pl.ds(rb * RB, RB), :], xsems.at[rb])
    c_w = [cp(i, wqkv_hbm.at[:, i * D:(i + 1) * D], wqkv.at[i]) for i in range(3)]
    c_bw = []
    for w, src in enumerate((wq_hbm, wk_hbm, wv_hbm)):
        su = src.bitcast(jnp.uint32)
        c_bw.append([cp(3 + w, su.at[:, hp, :], uw.at[w, hp]) for hp in range(HB // 2)])
    c_awo = cp(6, awo_hbm, awo)
    c_bwo = cp(7, bwo_hbm, bwo)
    c_bx = cp(8, bx_hbm, xb)
    c_mem = cp(9, mem0_hbm, mem0v)
    c_oa = cp(10, stage_a, out_hbm.at[:, 0:D])
    c_w[0].start()
    cx(0).start()
    for rb in range(1, NRB):
        cx(rb).start()
    c_w[1].start()
    c_w[2].start()

    qscale = (DA ** -0.5) * LOG2E
    c_w[0].wait()

    def q_body(rb, carry):
        cx(rb).wait()
        r0 = pl.multiple_of(rb * RB, RB)
        x = xa[pl.ds(r0, RB), :]
        GW = cfg["GW"]
        for g0 in range(0, 8, GW):
            q = (_dot(x, wqkv[0, :, g0 * 128:(g0 + GW) * 128]) * qscale).astype(bf16)
            for gg in range(GW):
                g = g0 + gg
                qg = q[:, gg * 128:(gg + 1) * 128].T
                qt[g, :, pl.ds(r0, RB)] = qg
                qf = qg.astype(f32)
                q2buf[g * 4:(g + 1) * 4, pl.ds(r0, RB)] = jnp.sum((qf * qf).reshape(4, DA, RB), axis=1)
        return carry
    lax.fori_loop(0, NRB, q_body, 0)

    def start_big():
        for cs in c_bw:
            for c in cs:
                c.start()
        for c in (c_awo, c_bwo, c_bx, c_mem):
            c.start()
    if cfg['dmapos'] == 'q':
        start_big()
    c_w[1].wait()
    c_w[2].wait()

    def kv_body(rb, carry):
        r0 = pl.multiple_of(rb * RB, RB)
        x = xa[pl.ds(r0, RB), :]
        GW = cfg["GW"]
        for g0 in range(0, 8, GW):
            k = _dot(x, wqkv[1, :, g0 * 128:(g0 + GW) * 128]).astype(bf16)
            for gg in range(GW):
                g = g0 + gg
                kg = k[:, gg * 128:(gg + 1) * 128]
                kk[g, pl.ds(r0, RB), :] = kg
                kf = kg.T.astype(f32)
                k2 = jnp.sum((kf * kf).reshape(4, DA, RB), axis=1)
                km = k2[:, 0:128]
                for t in range(1, RB // 128):
                    km = jnp.maximum(km, k2[:, t * 128:(t + 1) * 128])
                kmpart[rb, g * 4:(g + 1) * 4, :] = km
        for g0 in range(0, 8, GW):
            v = _dot(x, wqkv[2, :, g0 * 128:(g0 + GW) * 128]).astype(bf16)
            for gg in range(GW):
                g = g0 + gg
                vt[g * 128:(g + 1) * 128, pl.ds(r0, RB)] = v[:, gg * 128:(gg + 1) * 128].T
        return carry
    lax.fori_loop(0, NRB, kv_body, 0)

    kmx[...] = jnp.broadcast_to(jnp.max(jnp.max(kmpart[...], axis=0), axis=1, keepdims=True), (HA, 128))

    NB = S // NQ
    NIT = HA * NB
    NKC = S // KC
    NBODY = NIT // UN
    rowj = lax.broadcasted_iota(jnp.int32, (128, NQ), 0) // DA

    def kchunk(g, kc0, n):
        return kk[g, pl.ds(kc0, n), :]

    def setup_q(i, slot):
        h = i // NB
        qb = i % NB
        g = h // 4
        j = h % 4
        q0 = pl.multiple_of(qb * NQ, NQ)
        qv = qt[g, :, pl.ds(q0, NQ)]
        qm[slot] = jnp.where(rowj == j, qv, jnp.zeros_like(qv))

    if cfg['dmapos'] == 'v':
        start_big()
    setup_q(0, 0)

    def attn_body(ii, carry):
        gs, hs, q0s, ms = [], [], [], []
        for u in range(UN):
            i = UN * ii + u
            h = i // NB
            q0 = pl.multiple_of((i % NB) * NQ, NQ)
            hs.append(h)
            q0s.append(q0)
            gs.append(h // 4)
            if u > 0:
                setup_q(i, u)
            km = kmx[pl.ds(h, 1), :]
            bound = jnp.sqrt(q2buf[pl.ds(h, 1), pl.ds(q0, NQ)] * jnp.concatenate([km] * (NQ // 128), axis=1)) * 1.001
            ms.append(jnp.broadcast_to(bound, (8, NQ)))
        l8 = [None] * UN
        o = [None] * UN
        pst = {}
        for t in range(UN * NKC + SK):
            if t < UN * NKC:
                u, kc = divmod(t, NKC)
                s = _dot(kchunk(gs[u], kc * KC, KC), qm[u])
                p = jnp.exp2(s.reshape(KC // 8, 8, NQ) - ms[u][None])
                ps = jnp.sum(p, axis=0)
                l8[u] = ps if l8[u] is None else l8[u] + ps
                pst[t] = p.reshape(KC, NQ).astype(bf16)
                if u == 0 and kc == NKC - 1:
                    setup_q(jnp.minimum(UN * ii + UN, NIT - 1), 0)
            tt = t - SK
            if tt >= 0:
                u, kc = divmod(tt, NKC)
                hrow = pl.ds(pl.multiple_of(hs[u] * DA, DA), DA)
                oc = _dot(vt[hrow, kc * KC:(kc + 1) * KC], pst.pop(tt))
                o[u] = oc if o[u] is None else o[u] + oc
                if kc == NKC - 1:
                    l = jnp.sum(l8[u], axis=0, keepdims=True)
                    lbuf[pl.ds(hs[u], 1), pl.ds(q0s[u], NQ)] = l
                    ot[hrow, pl.ds(q0s[u], NQ)] = (o[u] * (1.0 / l)).astype(bf16)
        return carry
    lax.fori_loop(0, NBODY, attn_body, 0)

    def is_bad(lv):
        return jnp.logical_not(jnp.logical_and(lv > 2.0 ** -80, lv < 2.0 ** 80))
    nbad_all = jnp.sum(is_bad(lbuf[...]).astype(jnp.int32))

    @pl.when(nbad_all != 0)
    def _():
        def check_body(h, carry):
            nbad = jnp.sum(is_bad(lbuf[pl.ds(h, 1), :]).astype(jnp.int32))

            @pl.when(nbad != 0)
            def _():
                def fb_body(qb, c2):
                    q0 = pl.multiple_of(qb * NQ, NQ)
                    setup_q(h * NB + qb, 0)
                    g = h // 4
                    hrow = pl.ds(pl.multiple_of(h * DA, DA), DA)
                    s0 = _dot(kk[g, 0:1024], qm[0])
                    s1 = _dot(kk[g, 1024:2048], qm[0])
                    m = jnp.maximum(jnp.max(s0, axis=0, keepdims=True), jnp.max(s1, axis=0, keepdims=True))
                    p0 = jnp.exp2(s0 - m)
                    p1 = jnp.exp2(s1 - m)
                    l = jnp.sum(p0, axis=0, keepdims=True) + jnp.sum(p1, axis=0, keepdims=True)
                    oo = _dot(vt[hrow, 0:1024], p0.astype(bf16)) + _dot(vt[hrow, 1024:2048], p1.astype(bf16))
                    ot[hrow, pl.ds(q0, NQ)] = (oo * (1.0 / l)).astype(bf16)
                    return c2
                lax.fori_loop(0, NB, fb_body, 0)
            return carry
        lax.fori_loop(0, HA, check_body, 0)

    c_awo.wait()

    def oproj_body(rb, carry):
        r0 = pl.multiple_of(rb * RB, RB)
        stage_a[pl.ds(r0, RB), :] = _dot(ot[:, pl.ds(r0, RB)], awo[...], TN).astype(bf16)
        return carry
    lax.fori_loop(0, NRB, oproj_body, 0)
    c_oa.start()

    for cs in c_bw:
        for c in cs:
            c.wait()
    c_bwo.wait()
    c_bx.wait()
    c_mem.wait()

    bscale = DB ** -0.5
    row = lax.broadcasted_iota(jnp.int32, (L, L), 0)
    col = lax.broadcasted_iota(jnp.int32, (L, L), 1)
    mask = (row < M) | (row >= col)
    hcat[0:M, :] = mem0v[...].astype(f32)
    order = cfg["order"]

    def bw(w, h):
        x = uw[w, h // 2]
        if h % 2:
            x = x >> 16
        return pltpu.bitcast(x.astype(jnp.uint16), bf16)

    def seg_body(s, carry):
        r0 = pl.multiple_of(s * SEG, SEG)
        hcat[M:L, :] = xb[pl.ds(r0, SEG), :].astype(f32)
        hc = hcat[...]
        st = {}
        acc = [None]

        def Q(h): st['q', h] = _dot(hc, bw(0, h))
        def K(h): st['k', h] = _dot(hc, bw(1, h))
        def V(h): st['v', h] = _dot(hc, bw(2, h))

        def SC(h):
            sc = _dot(st.pop(('q', h)), st.pop(('k', h)).astype(bf16), NT) * bscale
            sc = jnp.where(mask, sc, -1e9)
            m = jnp.max(sc, axis=-1, keepdims=True)
            p = jnp.exp(sc - m)
            l = jnp.sum(p, axis=-1, keepdims=True)
            st['p', h] = p
            st['rl', h] = 1.0 / l

        def PV(h):
            oo = _dot(st.pop(('p', h)), st.pop(('v', h)).astype(bf16))
            st['o', h] = oo * st.pop(('rl', h))

        def O(h):
            po = _dot(st.pop(('o', h)), bwo[h])
            acc[0] = po if acc[0] is None else acc[0] + po
        fns = dict(Q=Q, K=K, V=V, SC=SC, PV=PV, O=O)
        for name, h in order:
            fns[name](h)
        accb = acc[0].astype(bf16)
        hcat[0:M, :] = accb[0:M].astype(f32)
        stage_b[pl.ds(r0, SEG), :] = accb[M:L]
        return carry

    NOB = cfg["NOB"]
    SPB = NSEG // NOB
    OR = SPB * SEG

    def c_ob(blk):
        r0 = pl.multiple_of(blk * OR, OR)
        return pltpu.make_async_copy(stage_b.at[pl.ds(r0, OR), :], out_hbm.at[pl.ds(r0, OR), D:2 * D], sems.at[11])

    def blk_body(blk, carry):
        UNB = cfg["UNB"]

        def segs(ss, c):
            for u in range(UNB):
                seg_body(ss * UNB + u, c)
            return c
        lax.fori_loop(blk * (SPB // UNB), (blk + 1) * (SPB // UNB), segs, 0)
        c_ob(blk).start()
        return carry
    lax.fori_loop(0, NOB, blk_body, 0)
    c_oa.wait()
    for blk in range(NOB):
        c_ob(blk).wait()


def _tail_order(d_o=6, ntail=(2, 4)):
    dq = [('Q', 0), ('K', 0), ('V', 0), ('SC', -1), ('PV', -2), ('O', -d_o)]
    out = []
    for i in range(HB):
        for name, off in dq:
            h = i + off
            if 0 <= h < HB:
                out.append((name, h))
    done = set(out)
    os_ = [('O', h) for h in range(HB) if ('O', h) not in done]
    t = [('SC', HB - 1)] + os_[:ntail[0]] + [('PV', HB - 2)] + os_[ntail[0]:ntail[1]] + [('PV', HB - 1)] + os_[ntail[1]:]
    return tuple(out + t)


CFG = dict(GW=1, dmapos='q', UNB=1, NQ=512, KC=256, SK=1, UN=4, RB=512, NOB=8, order=_tail_order())


@functools.partial(jax.jit, static_argnames=("B_seg_len",))
def pallas_concat_heads__softmax_full_mha__memory_aug_recurrent_mem_tr__prompt_kernel(
        A_x, A_wqkv, A_wo, B_x, B_mem0, B_Wq, B_Wk, B_Wv, B_Wo, B_seg_len):
    assert B_seg_len == SEG
    any_ = pl.BlockSpec(memory_space=pl.ANY)
    V = pltpu.VMEM
    cfg = CFG
    NQ, UN, RB = cfg["NQ"], cfg["UN"], cfg["RB"]
    scratch = [
        V((S, D), bf16), V((3, D, D), bf16), V((D, D), bf16),
        V((8, 128, S), bf16), V((8, S, 128), bf16), V((D, S), bf16), V((D, S), bf16),
        V((HA, S), f32), V((S // RB, HA, 128), f32), V((HA, 128), f32), V((HA, S), f32),
        V((UN, 128, NQ), bf16), V((S, D), bf16),
        V((S, D), bf16), V((8, D), bf16), V((3, HB // 2, D, DB), jnp.uint32),
        V((32, 128, D), bf16), V((L, D), f32), V((S, D), bf16),
        pltpu.SemaphoreType.DMA((S // RB,)),
        pltpu.SemaphoreType.DMA((12,)),
    ]
    out = pl.pallas_call(
        functools.partial(_kernel, cfg=cfg),
        out_shape=jax.ShapeDtypeStruct((S, 2 * D), bf16),
        in_specs=[any_] * 9,
        out_specs=any_,
        scratch_shapes=scratch,
        compiler_params=pltpu.CompilerParams(vmem_limit_bytes=124 * 2 ** 20),
    )(A_x.reshape(S, D), A_wqkv, A_wo, B_x.reshape(S, D), B_mem0.reshape(8, D), B_Wq, B_Wk, B_Wv, B_Wo)
    return out.reshape(1, S, 2 * D)
```

```python
import functools

import jax
import jax.numpy as jnp
from jax import lax
from jax.experimental import pallas as pl
from jax.experimental.pallas import tpu as pltpu

f32 = jnp.float32
bf16 = jnp.bfloat16
NN = (((1,), (0,)), ((), ()))
NT = (((1,), (1,)), ((), ()))
TN = (((0,), (0,)), ((), ()))
LOG2E = 1.4426950408889634

S, D = 2048, 1024
HA, DA = 32, 32
HB, DB, M, SEG = 32, 128, 8, 32
L = M + SEG
NSEG = S // SEG

RB = 512
OQ = 4
NQ = 512
KC = 128
SK = 2
UN = 2
NB = S // NQ
NIT = HA * NB
NKC = S // KC
NSLOT = UN * NKC + SK
assert NIT == UN * NSEG
L_MIN, L_MAX = 2.0 ** -60, 2.0 ** 60


def _dot(a, b, dn=NN):
    return lax.dot_general(a, b, dn, preferred_element_type=f32)


def _segment_order():
    order = []
    for i in range(HB):
        order += [("Q", i), ("A", i) if i < HB - 1 else None, ("K", i), ("SC", i - 1), ("V", i),
                  ("PV", i - 3), ("O", i - 6)]
    order = [op for op in order if op is not None and op[1] >= 0]
    order += [("SC", 31), ("A", 31), ("PV", 29), ("A", 32), ("O", 26), ("A", 33), ("PV", 30), ("PV", 31),
              ("O", 27), ("O", 28), ("O", 29), ("O", 30), ("O", 31)]
    assert NSLOT == 34 and len(order) == 6 * HB + NSLOT
    return tuple(order)


def _kernel(ax_hbm, wqkv_hbm, awo_hbm, bx_hbm, mem0_hbm, wq_hbm, wk_hbm, wv_hbm, bwo_hbm,
            out_hbm,
            xa, wqkv, awo, qt, kk, vt, ot, q2buf, kmpart, kmx, lbuf, qm, stage_a,
            xb, mem0v, uw, bwo, hcat, stage_b, xsems, sems):
    def cp(i, src, dst):
        return pltpu.make_async_copy(src, dst, sems.at[i])

    def c_x(rb):
        rows = pl.ds(rb * RB, RB)
        return pltpu.make_async_copy(ax_hbm.at[rows, :], xa.at[rows, :], xsems.at[rb])

    c_w = [cp(i, wqkv_hbm.at[:, i * D:(i + 1) * D], wqkv.at[i]) for i in range(3)]
    c_bw = []
    for w, src in enumerate((wq_hbm, wk_hbm, wv_hbm)):
        su = src.bitcast(jnp.uint32)
        c_bw += [cp(3 + w, su.at[:, hp, :], uw.at[w, hp]) for hp in range(HB // 2)]
    c_awo = cp(6, awo_hbm, awo)
    c_bwo = cp(7, bwo_hbm, bwo)
    c_bx = cp(8, bx_hbm, xb)
    c_mem = cp(9, mem0_hbm, mem0v)
    c_ob = cp(11, stage_b, out_hbm.at[:, D:2 * D])

    def c_oa(r0, n):
        return pltpu.make_async_copy(stage_a.at[pl.ds(r0, n), :], out_hbm.at[pl.ds(r0, n), 0:D], sems.at[10])

    c_w[0].start()
    for rb in range(S // RB):
        c_x(rb).start()
    c_w[1].start()
    c_w[2].start()

    qscale = (DA ** -0.5) * LOG2E
    c_w[0].wait()

    def q_body(rb, carry):
        c_x(rb).wait()
        r0 = pl.multiple_of(rb * RB, RB)
        x = xa[pl.ds(r0, RB), :]
        for g in range(8):
            qg = (_dot(x, wqkv[0, :, g * 128:(g + 1) * 128]) * qscale).astype(bf16).T
            qt[g, :, pl.ds(r0, RB)] = qg
            qf = qg.astype(f32)
            q2buf[g * 4:(g + 1) * 4, pl.ds(r0, RB)] = jnp.sum((qf * qf).reshape(4, DA, RB), axis=1)

        @pl.when(rb == 1)
        def _():
            for c in c_bw + [c_awo, c_bwo, c_bx, c_mem]:
                c.start()
        return carry
    lax.fori_loop(0, S // RB, q_body, 0)

    c_w[1].wait()
    c_w[2].wait()

    def kv_body(rb, carry):
        r0 = pl.multiple_of(rb * RB, RB)
        x = xa[pl.ds(r0, RB), :]
        for g in range(8):
            kg = _dot(x, wqkv[1, :, g * 128:(g + 1) * 128]).astype(bf16)
            kk[g, pl.ds(r0, RB), :] = kg
            kf = kg.T.astype(f32)
            k2 = jnp.sum((kf * kf).reshape(4, DA, RB), axis=1)
            km = k2[:, 0:128]
            for t in range(1, RB // 128):
                km = jnp.maximum(km, k2[:, t * 128:(t + 1) * 128])
            kmpart[rb, g * 4:(g + 1) * 4, :] = km
        for g in range(8):
            vt[g * 128:(g + 1) * 128, pl.ds(r0, RB)] = _dot(x, wqkv[2, :, g * 128:(g + 1) * 128]).astype(bf16).T
        return carry
    lax.fori_loop(0, S // RB, kv_body, 0)

    kmx[...] = jnp.broadcast_to(jnp.max(jnp.max(kmpart[...], axis=0), axis=1, keepdims=True), (HA, 128))

    rowj = lax.broadcasted_iota(jnp.int32, (128, NQ), 0) // DA

    def setup_q(i, slot):
        h = i // NB
        q0 = pl.multiple_of((i % NB) * NQ, NQ)
        qv = qt[h // 4, :, pl.ds(q0, NQ)]
        qm[slot] = jnp.where(rowj == h % 4, qv, jnp.zeros_like(qv))

    setup_q(0, 0)

    def attn_slots(ii):
        gs, hs, q0s, nms = [], [], [], []
        for u in range(UN):
            i = UN * ii + u
            h = i // NB
            q0 = pl.multiple_of((i % NB) * NQ, NQ)
            hs.append(h)
            q0s.append(q0)
            gs.append(h // 4)
            if u > 0:
                setup_q(i, u)
            km = kmx[pl.ds(h, 1), :]
            bound = jnp.sqrt(q2buf[pl.ds(h, 1), pl.ds(q0, NQ)] * jnp.concatenate([km] * (NQ // 128), axis=1)) * 1.001
            nms.append(jnp.broadcast_to(-bound, (8, NQ)))
        l8 = [None] * UN
        o = [None] * UN
        l8_hist = {}
        p_stash = {}

        def slot(t):
            if t < UN * NKC:
                u, kc = divmod(t, NKC)
                s = _dot(kk[gs[u], kc * KC:(kc + 1) * KC, :], qm[u])
                nm = nms[u] if kc == 0 else jnp.minimum(nms[u], l8_hist[u, kc - 1])
                p = jnp.exp2(s.reshape(KC // 8, 8, NQ) + nm[None])
                ps = jnp.sum(p, axis=0)
                l8[u] = ps if l8[u] is None else l8[u] + ps
                l8_hist[u, kc] = l8[u]
                p_stash[t] = p.reshape(KC, NQ).astype(bf16)
                if u == 0 and kc == NKC - 1:
                    setup_q(jnp.minimum(UN * ii + UN, NIT - 1), 0)
            tt = t - SK
            if tt >= 0:
                u, kc = divmod(tt, NKC)
                hrow = pl.ds(pl.multiple_of(hs[u] * DA, DA), DA)
                oc = _dot(vt[hrow, kc * KC:(kc + 1) * KC], p_stash.pop(tt))
                o[u] = oc if o[u] is None else o[u] + oc
                if kc == NKC - 1:
                    l = jnp.sum(l8[u], axis=0, keepdims=True)
                    lbuf[pl.ds(hs[u], 1), pl.ds(q0s[u], NQ)] = l
                    ot[hrow, pl.ds(q0s[u], NQ)] = (o[u] * (1.0 / l)).astype(bf16)
        return slot

    for c in c_bw + [c_bwo, c_bx, c_mem]:
        c.wait()

    bscale = DB ** -0.5
    row = lax.broadcasted_iota(jnp.int32, (L, L), 0)
    col = lax.broadcasted_iota(jnp.int32, (L, L), 1)
    mask = (row < M) | (row >= col)
    hcat[0:M, :] = mem0v[...].astype(f32)
    order = _segment_order()

    def bw(w, h):
        x = uw[w, h // 2]
        if h % 2:
            x = x >> 16
        return pltpu.bitcast(x.astype(jnp.uint16), bf16)

    def seg_body(s, carry):
        r0 = pl.multiple_of(s * SEG, SEG)
        hcat[M:L, :] = xb[pl.ds(r0, SEG), :].astype(f32)
        hc = hcat[...]
        st = {}
        acc = [None]

        def Q(h): st["q", h] = _dot(hc, bw(0, h))
        def K(h): st["k", h] = _dot(hc, bw(1, h))
        def V(h): st["v", h] = _dot(hc, bw(2, h))

        def SC(h):
            sc = _dot(st.pop(("q", h)), st.pop(("k", h)).astype(bf16), NT) * bscale
            sc = jnp.where(mask, sc, -1e9)
            m = jnp.max(sc, axis=-1, keepdims=True)
            p = jnp.exp(sc - m)
            st["p", h] = p
            st["rl", h] = 1.0 / jnp.sum(p, axis=-1, keepdims=True)

        def PV(h):
            st["o", h] = _dot(st.pop(("p", h)), st.pop(("v", h)).astype(bf16)) * st.pop(("rl", h))

        def O(h):
            po = _dot(st.pop(("o", h)), bwo[h])
            acc[0] = po if acc[0] is None else acc[0] + po

        fns = dict(Q=Q, K=K, V=V, SC=SC, PV=PV, O=O, A=attn_slots(s))
        for name, h in order:
            fns[name](h)
        accb = acc[0].astype(bf16)
        hcat[0:M, :] = accb[0:M].astype(f32)
        stage_b[pl.ds(r0, SEG), :] = accb[M:L]
        return carry
    lax.fori_loop(0, NSEG, seg_body, 0)
    c_ob.start()

    def is_bad(lv):
        return jnp.logical_not(jnp.logical_and(lv > L_MIN, lv < L_MAX))

    @pl.when(jnp.sum(is_bad(lbuf[...]).astype(jnp.int32)) != 0)
    def _():
        def check_head(h, carry):
            @pl.when(jnp.sum(is_bad(lbuf[pl.ds(h, 1), :]).astype(jnp.int32)) != 0)
            def _():
                def redo(qb, c2):
                    q0 = pl.multiple_of(qb * NQ, NQ)
                    setup_q(h * NB + qb, 0)
                    g = h // 4
                    hrow = pl.ds(pl.multiple_of(h * DA, DA), DA)
                    s0 = _dot(kk[g, 0:S // 2], qm[0])
                    s1 = _dot(kk[g, S // 2:S], qm[0])
                    m = jnp.maximum(jnp.max(s0, axis=0, keepdims=True), jnp.max(s1, axis=0, keepdims=True))
                    p0 = jnp.exp2(s0 - m)
                    p1 = jnp.exp2(s1 - m)
                    l = jnp.sum(p0, axis=0, keepdims=True) + jnp.sum(p1, axis=0, keepdims=True)
                    oo = _dot(vt[hrow, 0:S // 2], p0.astype(bf16)) + _dot(vt[hrow, S // 2:S], p1.astype(bf16))
                    ot[hrow, pl.ds(q0, NQ)] = (oo * (1.0 / l)).astype(bf16)
                    return c2
                lax.fori_loop(0, NB, redo, 0)
            return carry
        lax.fori_loop(0, HA, check_head, 0)

    c_awo.wait()
    RQ = RB // OQ

    def oproj_body(rb, carry):
        for qd in range(OQ):
            r0 = pl.multiple_of(rb * RB + qd * RQ, RQ)
            stage_a[pl.ds(r0, RQ), :] = _dot(ot[:, pl.ds(r0, RQ)], awo[...], TN).astype(bf16)
            c_oa(r0, RQ).start()
        return carry
    lax.fori_loop(0, S // RB, oproj_body, 0)

    for j in range(S // RQ):
        c_oa(j * RQ, RQ).wait()
    c_ob.wait()


@functools.partial(jax.jit, static_argnames=("B_seg_len",))
def pallas_concat_heads__softmax_full_mha__memory_aug_recurrent_mem_tr__prompt_kernel(
        A_x, A_wqkv, A_wo, B_x, B_mem0, B_Wq, B_Wk, B_Wv, B_Wo, B_seg_len):
    assert B_seg_len == SEG
    any_ = pl.BlockSpec(memory_space=pl.ANY)
    V = pltpu.VMEM
    scratch = [
        V((S, D), bf16), V((3, D, D), bf16), V((D, D), bf16),
        V((8, 128, S), bf16), V((8, S, 128), bf16), V((D, S), bf16), V((D, S), bf16),
        V((HA, S), f32), V((S // RB, HA, 128), f32), V((HA, 128), f32), V((HA, S), f32),
        V((UN, 128, NQ), bf16), V((S, D), bf16),
        V((S, D), bf16), V((M, D), bf16), V((3, HB // 2, D, DB), jnp.uint32),
        V((HB, DB, D), bf16), V((L, D), f32), V((S, D), bf16),
        pltpu.SemaphoreType.DMA((S // RB,)),
        pltpu.SemaphoreType.DMA((12,)),
    ]
    out = pl.pallas_call(
        _kernel,
        out_shape=jax.ShapeDtypeStruct((S, 2 * D), bf16),
        in_specs=[any_] * 9,
        out_specs=any_,
        scratch_shapes=scratch,
        compiler_params=pltpu.CompilerParams(vmem_limit_bytes=124 * 2 ** 20),
    )(A_x.reshape(S, D), A_wqkv, A_wo, B_x.reshape(S, D), B_mem0.reshape(M, D), B_Wq, B_Wk, B_Wv, B_Wo)
    return out.reshape(1, S, 2 * D)
```

```python
import functools

import jax
import jax.numpy as jnp
from jax import lax
from jax.experimental import pallas as pl
from jax.experimental.pallas import tpu as pltpu

f32 = jnp.float32
bf16 = jnp.bfloat16
NN = (((1,), (0,)), ((), ()))
NT = (((1,), (1,)), ((), ()))
TN = (((0,), (0,)), ((), ()))
LOG2E = 1.4426950408889634

S, D = 2048, 1024
HA, DA = 32, 32
HB, DB, M, SEG = 32, 128, 8, 32
L = M + SEG
NSEG = S // SEG

RB = 512
OB = 1024
RQ = 128
NQ = 512
KC = 128
SK = 2
UN = 2
NB = S // NQ
NIT = HA * NB
NKC = S // KC
NSLOT = UN * NKC + SK
assert NIT == UN * NSEG
L_MIN, L_MAX = 2.0 ** -60, 2.0 ** 60


def _dot(a, b, dn=NN):
    return lax.dot_general(a, b, dn, preferred_element_type=f32)


_ORDER_TEXT = """
Q0 A0 K0 V0 Q1 A1 K1 SC0 Q2 A2 SC1 K2 V1 V2 Q3 A3 K3 SC2 Q4 V3 PV0 A4 K4 SC3 V4 PV1 Q5 A5 K5 SC4 V5 PV2 Q6 A6
SC5 K6 V6 PV3 O0 Q7 A7 K7 SC6 V7 PV4 O1 Q8 A8 K8 SC7 V8 PV5 O2 Q9 PV6 A9 K9 SC8 V9 O3 Q10 A10 K10 SC9 V10 O4 PV7
Q11 A11 K11 SC10 V11 PV8 O5 Q12 A12 K12 O6 SC11 V12 PV9 Q13 A13 K13 SC12 V13 PV10 O7 Q14 A14 K14 SC13 V14 PV11
O8 Q15 A15 K15 SC14 V15 O9 Q16 A16 K16 PV12 SC15 V16 PV13 O10 Q17 A17 K17 SC16 V17 PV14 O11 Q18 A18 K18 SC17 V18
PV15 O12 Q19 K19 A19 SC18 V19 PV16 O13 Q20 A20 K20 SC19 V20 PV17 O14 Q21 A21 K21 SC20 V21 PV18 O15 Q22 A22 K22
SC21 V22 O16 PV19 Q23 A23 K23 O17 SC22 V23 PV20 Q24 A24 K24 SC23 V24 PV21 O18 Q25 A25 K25 SC24 V25 PV22 O19 Q26
A26 K26 V26 SC25 PV23 O20 Q27 A27 A28 SC26 PV24 K27 O21 V27 Q28 K28 PV25 SC27 O22 V28 Q29 A29 K29 PV26 SC28 O23
V29 Q30 A30 K30 SC29 PV27 Q31 V30 PV28 K31 O24 SC30 O25 V31 SC31 A31 PV29 A32 O26 A33 PV30 PV31 O28 O29 O30 O31
O27
"""


def _segment_order():
    order = tuple((tok.rstrip("0123456789"), int(tok.lstrip("AKOPQSCV"))) for tok in _ORDER_TEXT.split())
    pos = {op: i for i, op in enumerate(order)}
    assert len(pos) == len(order) == 6 * HB + NSLOT
    for h in range(HB):
        assert max(pos["Q", h], pos["K", h]) < pos["SC", h] < pos["PV", h] < pos["O", h] and pos["V", h] < pos["PV", h]
    assert all(pos["A", t] < pos["A", t + 1] for t in range(NSLOT - 1))
    return order


def _kernel(ax_hbm, wqkv_hbm, awo_hbm, bx_hbm, mem0_hbm, wq_hbm, wk_hbm, wv_hbm, bwo_hbm,
            out_hbm,
            xa, wqkv, awo, qt, kk, vt, ot, q2buf, kmpart, kmx, lbuf, qm, stage_a,
            xb, mem0v, uw, bwo, hcat, stage_b, xsems, sems):
    def cp(i, src, dst):
        return pltpu.make_async_copy(src, dst, sems.at[i])

    def c_x(rb):
        rows = pl.ds(rb * RB, RB)
        return pltpu.make_async_copy(ax_hbm.at[rows, :], xa.at[rows, :], xsems.at[rb])

    c_w = [cp(i, wqkv_hbm.at[:, i * D:(i + 1) * D], wqkv.at[i]) for i in range(3)]
    c_bw = []
    for w, src in enumerate((wq_hbm, wk_hbm, wv_hbm)):
        su = src.bitcast(jnp.uint32)
        c_bw += [cp(3 + w, su.at[:, hp, :], uw.at[w, hp]) for hp in range(HB // 2)]
    c_awo = cp(6, awo_hbm, awo)
    c_bwo = cp(7, bwo_hbm, bwo)
    c_bx = cp(8, bx_hbm, xb)
    c_mem = cp(9, mem0_hbm, mem0v)
    c_ob = cp(11, stage_b, out_hbm.at[:, D:2 * D])

    def c_oa(r0, n):
        return pltpu.make_async_copy(stage_a.at[pl.ds(r0, n), :], out_hbm.at[pl.ds(r0, n), 0:D], sems.at[10])

    c_w[0].start()
    for rb in range(S // RB):
        c_x(rb).start()
    c_w[1].start()
    c_w[2].start()

    qscale = (DA ** -0.5) * LOG2E
    c_w[0].wait()

    def q_body(rb, carry):
        c_x(rb).wait()
        r0 = pl.multiple_of(rb * RB, RB)
        x = xa[pl.ds(r0, RB), :]
        for g in range(8):
            qg = (_dot(x, wqkv[0, :, g * 128:(g + 1) * 128]) * qscale).astype(bf16).T
            qt[g, :, pl.ds(r0, RB)] = qg
            qf = qg.astype(f32)
            q2buf[g * 4:(g + 1) * 4, pl.ds(r0, RB)] = jnp.sum((qf * qf).reshape(4, DA, RB), axis=1)

        @pl.when(rb == 1)
        def _():
            for c in c_bw + [c_awo, c_bwo, c_bx, c_mem]:
                c.start()
        return carry
    lax.fori_loop(0, S // RB, q_body, 0)

    c_w[1].wait()
    c_w[2].wait()

    def kv_body(rb, carry):
        r0 = pl.multiple_of(rb * RB, RB)
        x = xa[pl.ds(r0, RB), :]
        for g in range(8):
            kg = _dot(x, wqkv[1, :, g * 128:(g + 1) * 128]).astype(bf16)
            kk[g, pl.ds(r0, RB), :] = kg
            kf = kg.T.astype(f32)
            k2 = jnp.sum((kf * kf).reshape(4, DA, RB), axis=1)
            km = k2[:, 0:128]
            for t in range(1, RB // 128):
                km = jnp.maximum(km, k2[:, t * 128:(t + 1) * 128])
            kmpart[rb, g * 4:(g + 1) * 4, :] = km
        for g in range(8):
            vt[g * 128:(g + 1) * 128, pl.ds(r0, RB)] = _dot(x, wqkv[2, :, g * 128:(g + 1) * 128]).astype(bf16).T
        return carry
    lax.fori_loop(0, S // RB, kv_body, 0)

    kmx[...] = jnp.broadcast_to(jnp.max(jnp.max(kmpart[...], axis=0), axis=1, keepdims=True), (HA, 128))

    rowj = lax.broadcasted_iota(jnp.int32, (128, NQ), 0) // DA

    def setup_q(i, slot):
        h = i // NB
        q0 = pl.multiple_of((i % NB) * NQ, NQ)
        qv = qt[h // 4, :, pl.ds(q0, NQ)]
        qm[slot] = jnp.where(rowj == h % 4, qv, jnp.zeros_like(qv))

    setup_q(0, 0)

    def attn_slots(ii):
        gs, hs, q0s, nms = [], [], [], []
        for u in range(UN):
            i = UN * ii + u
            h = i // NB
            q0 = pl.multiple_of((i % NB) * NQ, NQ)
            hs.append(h)
            q0s.append(q0)
            gs.append(h // 4)
            if u > 0:
                setup_q(i, u)
            km = kmx[pl.ds(h, 1), :]
            bound = jnp.sqrt(q2buf[pl.ds(h, 1), pl.ds(q0, NQ)] * jnp.concatenate([km] * (NQ // 128), axis=1)) * 1.001
            nms.append(jnp.broadcast_to(-bound, (8, NQ)))
        l8 = [None] * UN
        o = [None] * UN
        l8_hist = {}
        p_stash = {}

        def slot(t):
            if t < UN * NKC:
                u, kc = divmod(t, NKC)
                s = _dot(kk[gs[u], kc * KC:(kc + 1) * KC, :], qm[u])
                nm = nms[u] if kc == 0 else jnp.minimum(nms[u], l8_hist[u, kc - 1])
                p = jnp.exp2(s.reshape(KC // 8, 8, NQ) + nm[None])
                ps = jnp.sum(p, axis=0)
                l8[u] = ps if l8[u] is None else l8[u] + ps
                l8_hist[u, kc] = l8[u]
                p_stash[t] = p.reshape(KC, NQ).astype(bf16)
                if u == 0 and kc == NKC - 1:
                    setup_q(jnp.minimum(UN * ii + UN, NIT - 1), 0)
            tt = t - SK
            if tt >= 0:
                u, kc = divmod(tt, NKC)
                hrow = pl.ds(pl.multiple_of(hs[u] * DA, DA), DA)
                oc = _dot(vt[hrow, kc * KC:(kc + 1) * KC], p_stash.pop(tt))
                o[u] = oc if o[u] is None else o[u] + oc
                if kc == NKC - 1:
                    l = jnp.sum(l8[u], axis=0, keepdims=True)
                    lbuf[pl.ds(hs[u], 1), pl.ds(q0s[u], NQ)] = l
                    ot[hrow, pl.ds(q0s[u], NQ)] = (o[u] * (1.0 / l)).astype(bf16)
        return slot

    for c in c_bw + [c_bwo, c_bx, c_mem]:
        c.wait()

    bscale = DB ** -0.5
    row = lax.broadcasted_iota(jnp.int32, (L, L), 0)
    col = lax.broadcasted_iota(jnp.int32, (L, L), 1)
    mask = (row < M) | (row >= col)
    hcat[0:M, :] = mem0v[...].astype(f32)
    order = _segment_order()

    def bw(w, h):
        x = uw[w, h // 2]
        if h % 2:
            x = x >> 16
        return pltpu.bitcast(x.astype(jnp.uint16), bf16)

    def seg_body(s, carry):
        r0 = pl.multiple_of(s * SEG, SEG)
        hcat[M:L, :] = xb[pl.ds(r0, SEG), :].astype(f32)
        hc = hcat[...]
        st = {}
        acc = [None]

        def Q(h): st["q", h] = _dot(hc, bw(0, h))
        def K(h): st["k", h] = _dot(hc, bw(1, h))
        def V(h): st["v", h] = _dot(hc, bw(2, h))

        def SC(h):
            sc = _dot(st.pop(("q", h)), st.pop(("k", h)).astype(bf16), NT) * bscale
            sc = jnp.where(mask, sc, -1e9)
            m = jnp.max(sc, axis=-1, keepdims=True)
            p = jnp.exp(sc - m)
            st["p", h] = p
            st["rl", h] = 1.0 / jnp.sum(p, axis=-1, keepdims=True)

        def PV(h):
            st["o", h] = _dot(st.pop(("p", h)), st.pop(("v", h)).astype(bf16)) * st.pop(("rl", h))

        def O(h):
            po = _dot(st.pop(("o", h)), bwo[h])
            acc[0] = po if acc[0] is None else acc[0] + po

        fns = dict(Q=Q, K=K, V=V, SC=SC, PV=PV, O=O, A=attn_slots(s))
        for name, h in order:
            fns[name](h)
        accb = acc[0].astype(bf16)
        hcat[0:M, :] = accb[0:M].astype(f32)
        stage_b[pl.ds(r0, SEG), :] = accb[M:L]
        return carry
    lax.fori_loop(0, NSEG, seg_body, 0)
    c_ob.start()

    def is_bad(lv):
        return jnp.logical_not(jnp.logical_and(lv > L_MIN, lv < L_MAX))

    @pl.when(jnp.sum(is_bad(lbuf[...]).astype(jnp.int32)) != 0)
    def _():
        def check_head(h, carry):
            @pl.when(jnp.sum(is_bad(lbuf[pl.ds(h, 1), :]).astype(jnp.int32)) != 0)
            def _():
                def redo(qb, c2):
                    q0 = pl.multiple_of(qb * NQ, NQ)
                    setup_q(h * NB + qb, 0)
                    g = h // 4
                    hrow = pl.ds(pl.multiple_of(h * DA, DA), DA)
                    s0 = _dot(kk[g, 0:S // 2], qm[0])
                    s1 = _dot(kk[g, S // 2:S], qm[0])
                    m = jnp.maximum(jnp.max(s0, axis=0, keepdims=True), jnp.max(s1, axis=0, keepdims=True))
                    p0 = jnp.exp2(s0 - m)
                    p1 = jnp.exp2(s1 - m)
                    l = jnp.sum(p0, axis=0, keepdims=True) + jnp.sum(p1, axis=0, keepdims=True)
                    oo = _dot(vt[hrow, 0:S // 2], p0.astype(bf16)) + _dot(vt[hrow, S // 2:S], p1.astype(bf16))
                    ot[hrow, pl.ds(q0, NQ)] = (oo * (1.0 / l)).astype(bf16)
                    return c2
                lax.fori_loop(0, NB, redo, 0)
            return carry
        lax.fori_loop(0, HA, check_head, 0)

    c_awo.wait()

    def oproj_body(rb, carry):
        for qd in range(OB // RQ):
            r0 = pl.multiple_of(rb * OB + qd * RQ, RQ)
            stage_a[pl.ds(r0, RQ), :] = _dot(ot[:, pl.ds(r0, RQ)], awo[...], TN).astype(bf16)
            c_oa(r0, RQ).start()
        return carry
    lax.fori_loop(0, S // OB, oproj_body, 0)

    for j in range(S // RQ):
        c_oa(j * RQ, RQ).wait()
    c_ob.wait()


@functools.partial(jax.jit, static_argnames=("B_seg_len",))
def pallas_concat_heads__softmax_full_mha__memory_aug_recurrent_mem_tr__prompt_kernel(
        A_x, A_wqkv, A_wo, B_x, B_mem0, B_Wq, B_Wk, B_Wv, B_Wo, B_seg_len):
    assert B_seg_len == SEG
    any_ = pl.BlockSpec(memory_space=pl.ANY)
    V = pltpu.VMEM
    scratch = [
        V((S, D), bf16), V((3, D, D), bf16), V((D, D), bf16),
        V((8, 128, S), bf16), V((8, S, 128), bf16), V((D, S), bf16), V((D, S), bf16),
        V((HA, S), f32), V((S // RB, HA, 128), f32), V((HA, 128), f32), V((HA, S), f32),
        V((UN, 128, NQ), bf16), V((S, D), bf16),
        V((S, D), bf16), V((M, D), bf16), V((3, HB // 2, D, DB), jnp.uint32),
        V((HB, DB, D), bf16), V((L, D), f32), V((S, D), bf16),
        pltpu.SemaphoreType.DMA((S // RB,)),
        pltpu.SemaphoreType.DMA((12,)),
    ]
    out = pl.pallas_call(
        _kernel,
        out_shape=jax.ShapeDtypeStruct((S, 2 * D), bf16),
        in_specs=[any_] * 9,
        out_specs=any_,
        scratch_shapes=scratch,
        compiler_params=pltpu.CompilerParams(vmem_limit_bytes=96 * 2 ** 20),
    )(A_x.reshape(S, D), A_wqkv, A_wo, B_x.reshape(S, D), B_mem0.reshape(M, D), B_Wq, B_Wk, B_Wv, B_Wo)
    return out.reshape(1, S, 2 * D)
```
